```python
import os as _os
_os.environ.setdefault('JAX_PLATFORMS', 'cpu')
import jax
import jax.numpy as jnp

def _softmax(x, axis=-1):
    return jax.nn.softmax(x, axis=axis)

def _gelu(x):
    return jax.nn.gelu(x, approximate=True)

def _silu(x):
    return jax.nn.silu(x)

def _sigmoid(x):
    return jax.nn.sigmoid(x)

def _layernorm(x, axis=-1, eps=1e-05):
    m = jnp.mean(x, axis=axis, keepdims=True)
    v = jnp.var(x, axis=axis, keepdims=True)
    return (x - m) / jnp.sqrt(v + eps)

def _scatter_add(tgt, idx, src, axis=0):
    return tgt.at[idx].add(src)

def _segment_sum(src, seg, n):
    return jax.ops.segment_sum(src, seg, n)

class _Rng:

    def __init__(self, key):
        self._k = key

    def _next(self):
        self._k, sub = jax.random.split(self._k)
        return sub

    def normal(self, shape):
        return jax.random.normal(self._next(), shape, dtype=jnp.bfloat16)

    def randint(self, lo, hi, shape):
        return jax.random.randint(self._next(), shape, lo, hi, dtype=jnp.int32)

    def uniform(self, shape, lo=0.0, hi=1.0):
        return jax.random.uniform(self._next(), shape, jnp.bfloat16, lo, hi)

    def permutation(self, n):
        return jax.random.permutation(self._next(), n)
kernel_name = 'standalone__conformer_conv_module__speech'

def setup_inputs():
    _rng = _Rng(jax.random.key(int.from_bytes(__import__("os").urandom(4), "little")))
    _w = lambda a: (lambda t: t.astype(jnp.bfloat16) if jnp.issubdtype(t.dtype, jnp.floating) else t)(jnp.asarray(a))
    B, T, D, K = (2, 4000, 512, 15)
    return {'x': _w((lambda *s: _rng.normal(s) * 0.2)(B, T, D)), 'w_pw1': _w((lambda *s: _rng.normal(s) * 0.2)(D, 2 * D)), 'dw': _w((lambda *s: _rng.normal(s) * 0.05)(K, D)), 'w_pw2': _w((lambda *s: _rng.normal(s) * 0.05)(D, D))}

def reference(x, w_pw1, dw, w_pw2):
    B, T, D = x.shape
    K = dw.shape[0]
    h = x @ w_pw1
    a, b = (h[..., :D].copy(), h[..., D:].copy())
    h = a * _sigmoid(b)
    pad = K // 2
    hp = jnp.pad(h, ((0, 0), (pad, pad), (0, 0)))
    out = jnp.zeros_like(h)
    for i in range(K):
        out = out + hp[:, i:i + T, :] * dw[i][None, None, :]
    return _silu(out) @ w_pw2
```

```python
import functools
import os
import jax
import jax.numpy as jnp
import jax.experimental.pallas as pl
import jax.experimental.pallas.tpu as pltpu

LANES = 128
SKEW = 16
GAP = 8

CH = tuple(int(v) for v in os.environ.get("K_CH", "400,400,400,400,400,400,400,400,400,240,160").split(","))
NA = int(os.environ.get("K_NA", 2))
GROUPS = os.environ.get("K_GROUPS", "a0,g0,x0|a1,g1|a2,g2,a3,g3|x1,dw,w2")
PRO = os.environ.get("K_PRO", "W m1p:0.0 W m1p:0.1 W m1p:0.23 W T m1:1 TH:1 cm2:1 cm2x:0").split()
FLUSH = tuple(int(v) for v in os.environ.get("K_FL", "4,7,8,9,10").split(","))


def _kernel(x_hbm, w1_hbm, dw_hbm, w2_hbm, o_hbm,
            x_v, o_v, w1_v, w2_v, dw_v, tap_v, tap2_v, h_buf,
            sem_in, sem_xr, sem_o, *, B, T, D, K):
    NL = D // LANES
    pad = K // 2
    f32 = jnp.float32
    bf16 = jnp.bfloat16
    u32 = jnp.uint32
    N = len(CH)
    ends = [sum(CH[:i + 1]) for i in range(N)]
    starts = [0] + ends[:-1]
    lo = [max(s - SKEW, 0) for s in starts]
    hi = [e - SKEW for e in ends[:-1]] + [T]
    EA = ends[NA - 1]

    def x_copy(b, r0, r1, sem):
        return pltpu.make_async_copy(
            x_hbm.at[b, pl.ds(r0, r1 - r0), :], x_v.at[b, pl.ds(r0, r1 - r0), :], sem)

    def w1_copy(j, sem):
        return pltpu.make_async_copy(
            w1_hbm.at[:, pl.ds(j * LANES, LANES)], w1_v.at[j], sem)

    def w2_copy(j, sem):
        return pltpu.make_async_copy(
            w2_hbm.at[:, pl.ds(j * LANES, LANES)], w2_v.at[j], sem)

    groups = []
    for gi, g in enumerate(GROUPS.split("|")):
        sem = sem_in.at[gi]
        cps = []
        for it in g.split(","):
            if it[0] == "a":
                cps.append(w1_copy(int(it[1:]), sem))
            elif it[0] == "g":
                cps.append(w1_copy(NL + int(it[1:]), sem))
            elif it[0] == "x":
                i = int(it[1:])
                cps.append(x_copy(0, starts[i], ends[i], sem))
            elif it == "dw":
                cps.append(pltpu.make_async_copy(dw_hbm, dw_v, sem))
            elif it == "w2":
                cps += [w2_copy(j, sem) for j in range(NL)]
        groups.append(cps)
    G = len(groups)
    x_head1 = x_copy(1, 0, EA, sem_in.at[G])

    def x_rest(b):
        return x_copy(b, EA, T, sem_xr.at[b])

    NFIRST = min(3, G)
    for g in groups[:NFIRST]:
        for cp in g:
            cp.start()

    h_buf[:, 0:GAP, :] = jnp.zeros((NL, GAP, LANES), f32)
    h_buf[:, GAP + T:2 * GAP + T, :] = jnp.zeros((NL, GAP, LANES), f32)

    w1_u = w1_v.bitcast(u32)
    w2_u = w2_v.bitcast(u32)

    def w1t(j):
        return pltpu.bitcast(w1_u[j], bf16)

    def w2t(j):
        return pltpu.bitcast(w2_u[j], bf16)

    def m1(b, i, cs=range(NL)):
        r0, n = starts[i], CH[i]
        xs = x_v[b, r0:r0 + n, :]
        for c in cs:
            a = jnp.dot(xs, w1t(c), preferred_element_type=f32)
            g = jnp.dot(xs, w1t(NL + c), preferred_element_type=f32)
            h_buf[c, GAP + r0:GAP + r0 + n, :] = a + a * jnp.tanh(0.5 * g)

    def m1a(b, i, cs=range(NL)):
        r0, n = starts[i], CH[i]
        xs = x_v[b, r0:r0 + n, :]
        for c in cs:
            h_buf[c, GAP + r0:GAP + r0 + n, :] = jnp.dot(xs, w1t(c), preferred_element_type=f32)

    def m1g(b, i, cs=range(NL)):
        r0, n = starts[i], CH[i]
        xs = x_v[b, r0:r0 + n, :]
        for c in cs:
            g = jnp.dot(xs, w1t(NL + c), preferred_element_type=f32)
            a = h_buf[c, GAP + r0:GAP + r0 + n, :]
            h_buf[c, GAP + r0:GAP + r0 + n, :] = a + a * jnp.tanh(0.5 * g)

    def flush(b, r0, r1, j):
        pltpu.make_async_copy(
            o_v.at[b, j, pl.ds(r0, r1 - r0), :],
            o_hbm.at[b, pl.ds(r0, r1 - r0), pl.ds(j * LANES, LANES)],
            sem_o.at[0]).start()

    def cm2(b, i, tv=tap_v, flush_from=None):
        r0, n = lo[i], hi[i] - lo[i]
        h0 = GAP + r0 - pad
        ys = []
        for c in range(NL):
            acc = None
            for k in range(K):
                tap = tv[k, 0:1, c * LANES:(c + 1) * LANES]
                t = h_buf[c, h0 + k:h0 + k + n, :] * tap
                acc = t if acc is None else acc + t
            ys.append(acc + acc * jnp.tanh(acc))
        y = jnp.concatenate(ys, axis=1).astype(bf16)
        for j in range(NL):
            o = jnp.dot(y, w2t(j), preferred_element_type=f32)
            o_v[b, j, r0:r0 + n, :] = o.astype(bf16)
            if flush_from is not None:
                flush(b, flush_from, hi[i], j)

    wi = 0
    for p in PRO:
        if p == "W":
            for cp in groups[wi]:
                cp.wait()
            wi += 1
            if wi == 1:
                for g in groups[NFIRST:]:
                    for cp in g:
                        cp.start()
                for cp in [x_rest(0), x_head1, x_rest(1)]:
                    cp.start()
            continue
        if p == "T":
            dwf = dw_v[...].astype(f32) * 0.25
            for k in range(K):
                tap_v[k] = jnp.broadcast_to(dwf[k:k + 1, :], (8, D))
            continue
        op, arg = p.split(":")
        if op == "TH":
            r = GAP + starts[int(arg)]
            z = pltpu.bitcast(h_buf[0, r:r + 8, :], u32) & pltpu.bitcast(h_buf[0, 0:GAP, :], u32)
            z = jnp.concatenate([z] * NL, axis=1)
            dwf = dw_v[...].astype(f32) * 0.25
            for k in range(K):
                t = jnp.broadcast_to(dwf[k:k + 1, :], (8, D))
                tap2_v[k] = pltpu.bitcast(pltpu.bitcast(t, u32) | z, f32)
        elif op in ("m1", "a", "g"):
            {"m1": m1, "a": m1a, "g": m1g}[op](0, int(arg))
        elif op in ("m1p", "ap", "gp"):
            i, cs = arg.split(".")
            {"m1p": m1, "ap": m1a, "gp": m1g}[op](0, int(i), [int(c) for c in cs])
        elif op == "cm2":
            cm2(0, int(arg))
        elif op == "cm2x":
            cm2(0, int(arg), tap2_v)
    assert wi == G

    def body(b, carry):
        x_rest(b).wait()
        done = [0]

        def do_cm2(i):
            if i in FLUSH:
                cm2(b, i, flush_from=done[0])
                done[0] = hi[i]
            else:
                cm2(b, i)

        m1(b, NA)
        for i in range(NA, N):
            if i + 1 < N:
                m1(b, i + 1)
            do_cm2(i)

        @pl.when(b + 1 < B)
        def _():
            x_head1.wait()
            m1(1, 0)
            for i in range(NA):
                if i + 1 < NA:
                    m1(1, i + 1)
                cm2(1, i)
        return carry

    jax.lax.fori_loop(0, B, body, 0)
    pltpu.make_async_copy(o_hbm, o_hbm, sem_o.at[0]).wait()


@jax.jit
def pallas_standalone__conformer_conv_module__speech_kernel(x, w_pw1, dw, w_pw2):
    B, T, D = x.shape
    K = dw.shape[0]
    assert B == 2 and sum(CH) == T and all(c % 16 == 0 for c in CH) and (len(CH) - 1) in FLUSH
    NL = D // LANES
    kern = functools.partial(_kernel, B=B, T=T, D=D, K=K)
    return pl.pallas_call(
        kern,
        in_specs=[pl.BlockSpec(memory_space=pl.ANY)] * 4,
        out_specs=pl.BlockSpec(memory_space=pl.ANY),
        out_shape=jax.ShapeDtypeStruct((B, T, D), x.dtype),
        scratch_shapes=[
            pltpu.VMEM((B, T, D), x.dtype),
            pltpu.VMEM((B, NL, T, LANES), x.dtype),
            pltpu.VMEM((2 * NL, D, LANES), w_pw1.dtype),
            pltpu.VMEM((NL, D, LANES), w_pw2.dtype),
            pltpu.VMEM((K, D), dw.dtype),
            pltpu.VMEM((K, 8, D), jnp.float32),
            pltpu.VMEM((K, 8, D), jnp.float32),
            pltpu.VMEM((NL, T + 2 * GAP, LANES), jnp.float32),
            pltpu.SemaphoreType.DMA((len(GROUPS.split("|")) + 1,)),
            pltpu.SemaphoreType.DMA((B,)),
            pltpu.SemaphoreType.DMA((1,)),
        ],
        compiler_params=pltpu.CompilerParams(
            vmem_limit_bytes=64 * 1024 * 1024,
            disable_bounds_checks=True, disable_semaphore_checks=True),
    )(x, w_pw1, dw, w_pw2)
```

```python
import functools

import jax
import jax.numpy as jnp
import jax.experimental.pallas as pl
import jax.experimental.pallas.tpu as pltpu

LANES = 128
GAP = 8

R0 = 576
R1 = 1536
HP = 3008
PC = 1024
M1C = 384
CM2 = (512, 512, 512, 512, 512, 512, 368, 240, 192, 128)
LAST = 64


def _ranges(lo, hi, step):
    return [(r, min(r + step, hi)) for r in range(lo, hi, step)]


def _kernel(x_hbm, w1_hbm, dw_hbm, w2_hbm, o_hbm,
            x_v, o_v, w1_v, w2_v, dw_v, tap_v, acc_v, h_buf,
            sem_in, sem_o, *, B, T, D, K):
    NL = D // LANES
    pad = K // 2
    f32 = jnp.float32
    bf16 = jnp.bfloat16
    u32 = jnp.uint32

    def x_copy(b, r0, r1, k0, k1, sem):
        rows = pl.ds(r0, r1 - r0)
        cols = pl.ds(k0 * LANES, (k1 - k0) * LANES)
        return pltpu.make_async_copy(x_hbm.at[b, rows, cols], x_v.at[b, rows, cols], sem)

    def w1_copies(k0, k1, tiles, sem):
        rows = pl.ds(k0 * LANES, (k1 - k0) * LANES)
        return [pltpu.make_async_copy(w1_hbm.at[rows, pl.ds(j * LANES, LANES)],
                                      w1_v.at[j, rows, :], sem) for j in tiles]

    a_tiles = range(NL)
    g_tiles = range(NL, 2 * NL)
    g0 = w1_copies(0, 1, a_tiles, sem_in.at[0]) + [x_copy(0, 0, R0, 0, 1, sem_in.at[0])]
    g1 = w1_copies(0, 1, g_tiles, sem_in.at[1]) + [x_copy(0, R0, R1, 0, 1, sem_in.at[1])]
    g2 = [x_copy(0, R1, HP, 0, 1, sem_in.at[2]), x_copy(1, 0, HP, 0, 1, sem_in.at[2]),
          pltpu.make_async_copy(dw_hbm, dw_v, sem_in.at[2])]
    g3 = w1_copies(1, NL, range(2 * NL), sem_in.at[3]) + [
        pltpu.make_async_copy(w2_hbm.at[:, pl.ds(j * LANES, LANES)], w2_v.at[j], sem_in.at[3])
        for j in range(NL)]

    def x_rest(b):
        sem = sem_in.at[4 + b]
        return [x_copy(b, 0, HP, 1, NL, sem), x_copy(b, HP, T, 0, NL, sem)]

    for cp in g0 + g1 + g2 + g3 + x_rest(0) + x_rest(1):
        cp.start()

    h_buf[:, 0:GAP, :] = jnp.zeros((NL, GAP, LANES), f32)
    h_buf[:, GAP + T:2 * GAP + T, :] = jnp.zeros((NL, GAP, LANES), f32)

    w1_u = w1_v.bitcast(u32)
    w2_u = w2_v.bitcast(u32)

    def w1k(j, k0, k1):
        return pltpu.bitcast(w1_u[j, k0 * (LANES // 2):k1 * (LANES // 2), :], bf16)

    def w2t(j):
        return pltpu.bitcast(w2_u[j], bf16)

    def first_pass(b, r0, r1, tiles):
        xs = x_v[b, r0:r1, 0:LANES]
        w = jnp.concatenate([w1k(j, 0, 1) for j in tiles], axis=1)
        p = jnp.dot(xs, w, preferred_element_type=f32)
        for n, j in enumerate(tiles):
            acc_v[b, j, r0:r1, :] = p[:, n * LANES:(n + 1) * LANES]

    def glu_store(c, r0, r1, a, g):
        h_buf[c, GAP + r0:GAP + r1, :] = a + a * jnp.tanh(0.5 * g)

    def finish_pw1(b, r0, r1):
        xs = x_v[b, r0:r1, LANES:D]
        for c in range(NL):
            w = jnp.concatenate([w1k(c, 1, NL), w1k(NL + c, 1, NL)], axis=1)
            p = jnp.dot(xs, w, preferred_element_type=f32)
            glu_store(c, r0, r1,
                      p[:, :LANES] + acc_v[b, c, r0:r1, :],
                      p[:, LANES:] + acc_v[b, NL + c, r0:r1, :])

    def full_pw1(b, r0, r1):
        xs = x_v[b, r0:r1, :]
        for c in range(NL):
            a = jnp.dot(xs, w1k(c, 0, NL), preferred_element_type=f32)
            g = jnp.dot(xs, w1k(NL + c, 0, NL), preferred_element_type=f32)
            glu_store(c, r0, r1, a, g)

    def store_out(b, j, r0, r1, o):
        o_v[b, j, r0:r1, :] = o.astype(bf16)
        pltpu.make_async_copy(
            o_v.at[b, j, pl.ds(r0, r1 - r0), :],
            o_hbm.at[b, pl.ds(r0, r1 - r0), pl.ds(j * LANES, LANES)],
            sem_o.at[0]).start()

    def conv_pw2(b, r0, r1):
        n = r1 - r0
        h0 = GAP + r0 - pad
        ys = []
        for c in range(NL):
            acc = None
            for k in range(K):
                tap = tap_v[k, 0:1, c * LANES:(c + 1) * LANES]
                t = h_buf[c, h0 + k:h0 + k + n, :] * tap
                acc = t if acc is None else acc + t
            ys.append(acc + acc * jnp.tanh(acc))
        y = jnp.concatenate(ys, axis=1).astype(bf16)
        for j in range(NL):
            o = jnp.dot(y, w2t(j), preferred_element_type=f32)
            if r1 == T and j == NL - 1:
                store_out(b, j, r0, r1 - LAST, o[:n - LAST])
                store_out(b, j, r1 - LAST, r1, o[n - LAST:])
            else:
                store_out(b, j, r0, r1, o)

    def wait_all(cps):
        for cp in cps:
            cp.wait()

    def startup():
        wait_all(g0)
        first_pass(0, 0, R0, a_tiles)
        wait_all(g1)
        first_pass(0, R0, R1, a_tiles)
        first_pass(0, 0, R1, g_tiles)
        wait_all(g2)
        dwf = dw_v[...].astype(f32) * 0.25
        for k in range(K):
            tap_v[k] = jnp.broadcast_to(dwf[k:k + 1, :], (8, D))
        for b, lo in ((0, R1), (1, 0)):
            for r0, r1 in _ranges(lo, HP, PC):
                first_pass(b, r0, r1, a_tiles)
                first_pass(b, r0, r1, g_tiles)
        wait_all(g3)

    def body(b, carry):
        @pl.when(b == 0)
        def _():
            startup()

        wait_all(x_rest(b))
        for r0, r1 in _ranges(0, HP, M1C):
            finish_pw1(b, r0, r1)
        for r0, r1 in _ranges(HP, T, M1C):
            full_pw1(b, r0, r1)
        r0 = 0
        for n in CM2:
            conv_pw2(b, r0, r0 + n)
            r0 += n
        return carry

    jax.lax.fori_loop(0, B, body, 0)
    pltpu.make_async_copy(o_hbm, o_hbm, sem_o.at[0]).wait()


@jax.jit
def pallas_standalone__conformer_conv_module__speech_kernel(
    x: jax.Array,
    w_pw1: jax.Array,
    dw: jax.Array,
    w_pw2: jax.Array,
):
    B, T, D = x.shape
    K = dw.shape[0]
    assert B == 2 and sum(CM2) == T and D % LANES == 0 and K // 2 <= GAP
    NL = D // LANES
    kern = functools.partial(_kernel, B=B, T=T, D=D, K=K)
    return pl.pallas_call(
        kern,
        in_specs=[pl.BlockSpec(memory_space=pl.ANY)] * 4,
        out_specs=pl.BlockSpec(memory_space=pl.ANY),
        out_shape=jax.ShapeDtypeStruct((B, T, D), x.dtype),
        scratch_shapes=[
            pltpu.VMEM((B, T, D), x.dtype),
            pltpu.VMEM((B, NL, T, LANES), x.dtype),
            pltpu.VMEM((2 * NL, D, LANES), w_pw1.dtype),
            pltpu.VMEM((NL, D, LANES), w_pw2.dtype),
            pltpu.VMEM((K, D), dw.dtype),
            pltpu.VMEM((K, 8, D), jnp.float32),
            pltpu.VMEM((B, 2 * NL, HP, LANES), jnp.float32),
            pltpu.VMEM((NL, T + 2 * GAP, LANES), jnp.float32),
            pltpu.SemaphoreType.DMA((4 + B,)),
            pltpu.SemaphoreType.DMA((1,)),
        ],
        compiler_params=pltpu.CompilerParams(
            vmem_limit_bytes=100 * 1024 * 1024,
            disable_bounds_checks=True,
            disable_semaphore_checks=True),
    )(x, w_pw1, dw, w_pw2)
```

```python
import functools

import jax
import jax.numpy as jnp
import jax.experimental.pallas as pl
import jax.experimental.pallas.tpu as pltpu

LANES = 128
GAP = 8

R0 = 384
R1 = 832
HP = 3072
PC = 1024
M1C = 384
CM2 = (512, 512, 512, 512, 512, 512, 368, 240, 192, 128)
LAST = 64
NREP = 3


def _ranges(lo, hi, step):
    return [(r, min(r + step, hi)) for r in range(lo, hi, step)]


def _kernel(x_hbm, w1_hbm, dw_hbm, w2_hbm, o_hbm,
            x_v, o_v, w1_v, w2_v, w1_p, w2_p, dw_v, tap_v, acc_v, h_buf,
            sem_in, sem_o, *, B, T, D, K):
    NL = D // LANES
    pad = K // 2
    f32 = jnp.float32
    bf16 = jnp.bfloat16
    u32 = jnp.uint32

    def x_copy(b, r0, r1, k0, k1, sem):
        rows = pl.ds(r0, r1 - r0)
        cols = pl.ds(k0 * LANES, (k1 - k0) * LANES)
        return pltpu.make_async_copy(x_hbm.at[b, rows, cols], x_v.at[b, rows, cols], sem)

    def w1_copies(k0, k1, tiles, sem):
        rows = pl.ds(k0 * LANES, (k1 - k0) * LANES)
        return [pltpu.make_async_copy(w1_hbm.at[rows, pl.ds(j * LANES, LANES)],
                                      w1_v.at[j, rows, :], sem) for j in tiles]

    a_tiles = range(NL)
    g_tiles = range(NL, 2 * NL)
    g0 = w1_copies(0, 1, a_tiles, sem_in.at[0]) + [x_copy(0, 0, R0, 0, 1, sem_in.at[0])]
    g1 = w1_copies(0, 1, g_tiles, sem_in.at[1]) + [x_copy(0, R0, R1, 0, 1, sem_in.at[1])]
    g2 = [x_copy(0, R1, HP, 0, 1, sem_in.at[2]),
          pltpu.make_async_copy(dw_hbm, dw_v, sem_in.at[2])]
    g3 = [x_copy(1, 0, HP, 0, 1, sem_in.at[3])]
    g3 += w1_copies(1, NL, range(2 * NL), sem_in.at[3])
    g3 += [pltpu.make_async_copy(w2_hbm.at[:, pl.ds(j * LANES, LANES)], w2_v.at[j], sem_in.at[3])
           for j in range(NL)]

    def x_rest(b):
        sem = sem_in.at[4 + b]
        return [x_copy(b, 0, HP, 1, NL, sem), x_copy(b, HP, T, 0, NL, sem)]

    for cp in g0 + g1 + g2 + g3 + x_rest(0) + x_rest(1):
        cp.start()

    h_buf[:, 0:GAP, :] = jnp.zeros((NL, GAP, LANES), f32)
    h_buf[:, GAP + T:2 * GAP + T, :] = jnp.zeros((NL, GAP, LANES), f32)

    def w1k(j, k0, k1):
        return pltpu.bitcast(w1_p[j, k0 * (LANES // 2):k1 * (LANES // 2), :], bf16)

    def w2t(j):
        return pltpu.bitcast(w2_p[j], bf16)

    def first_pass(b, r0, r1, tiles):
        xs = x_v[b, r0:r1, 0:LANES]
        w = jnp.concatenate([w1_v[j, 0:LANES, :] for j in tiles], axis=1)
        p = jnp.dot(xs, w, preferred_element_type=f32)
        for n, j in enumerate(tiles):
            acc_v[b, j, r0:r1, :] = p[:, n * LANES:(n + 1) * LANES]
        return p

    def glu_store(c, r0, r1, a, g):
        h_buf[c, GAP + r0:GAP + r1, :] = a + a * jnp.tanh(0.5 * g)

    def finish_pw1(b, r0, r1):
        xs = x_v[b, r0:r1, LANES:D]
        for c in range(NL):
            w = jnp.concatenate([w1k(c, 1, NL), w1k(NL + c, 1, NL)], axis=1)
            p = jnp.dot(xs, w, preferred_element_type=f32)
            glu_store(c, r0, r1,
                      p[:, :LANES] + acc_v[b, c, r0:r1, :],
                      p[:, LANES:] + acc_v[b, NL + c, r0:r1, :])

    def full_pw1(b, r0, r1):
        xs = x_v[b, r0:r1, :]
        for c in range(NL):
            a = jnp.dot(xs, w1k(c, 0, NL), preferred_element_type=f32)
            g = jnp.dot(xs, w1k(NL + c, 0, NL), preferred_element_type=f32)
            glu_store(c, r0, r1, a, g)

    def store_out(b, j, r0, r1, o):
        o_v[b, j, r0:r1, :] = o.astype(bf16)
        pltpu.make_async_copy(
            o_v.at[b, j, pl.ds(r0, r1 - r0), :],
            o_hbm.at[b, pl.ds(r0, r1 - r0), pl.ds(j * LANES, LANES)],
            sem_o.at[0]).start()

    def conv_pw2(b, r0, r1):
        n = r1 - r0
        h0 = GAP + r0 - pad
        ys = []
        for c in range(NL):
            acc = None
            for k in range(K):
                tap = tap_v[k, 0:1, c * LANES:(c + 1) * LANES]
                t = h_buf[c, h0 + k:h0 + k + n, :] * tap
                acc = t if acc is None else acc + t
            ys.append(acc + acc * jnp.tanh(acc))
        y = jnp.concatenate(ys, axis=1).astype(bf16)
        for j in range(NL):
            o = jnp.dot(y, w2t(j), preferred_element_type=f32)
            if r1 == T and j == NL - 1:
                store_out(b, j, r0, r1 - LAST, o[:n - LAST])
                store_out(b, j, r1 - LAST, r1, o[n - LAST:])
            else:
                store_out(b, j, r0, r1, o)

    def wait_all(cps):
        for cp in cps:
            cp.wait()

    def startup():
        wait_all(g0)
        first_pass(0, 0, R0, a_tiles)
        wait_all(g1)
        first_pass(0, R0, R1, a_tiles)
        first_pass(0, 0, R1, g_tiles)
        wait_all(g2)
        dwf = dw_v[...].astype(f32) * 0.25
        for k in range(K):
            tap_v[k] = jnp.broadcast_to(dwf[k:k + 1, :], (8, D))
        for r0, r1 in _ranges(R1, HP, PC):
            first_pass(0, r0, r1, a_tiles)
            first_pass(0, r0, r1, g_tiles)
        wait_all(g3)
        todo = [(w1_v, w1_p, j) for j in range(2 * NL)] + [(w2_v, w2_p, j) for j in range(NL)]
        zero = pltpu.bitcast(h_buf[0, 0:1, :], u32)
        for r0, r1 in _ranges(0, HP, PC):
            for tiles in (a_tiles, g_tiles):
                p = first_pass(1, r0, r1, tiles)
                for q, (src, dst, j) in enumerate(todo[:NREP]):
                    pace = pltpu.bitcast(p[q * (D // 2):(q + 1) * (D // 2), 0:LANES], u32) & zero
                    dst[j] = pltpu.bitcast(src[j], u32) | pace
                todo = todo[NREP:]
        assert not todo

    def body(b, carry):
        @pl.when(b == 0)
        def _():
            startup()

        wait_all(x_rest(b))
        for r0, r1 in _ranges(0, HP, M1C):
            finish_pw1(b, r0, r1)
        for r0, r1 in _ranges(HP, T, M1C):
            full_pw1(b, r0, r1)
        r0 = 0
        for n in CM2:
            conv_pw2(b, r0, r0 + n)
            r0 += n
        return carry

    jax.lax.fori_loop(0, B, body, 0)
    pltpu.make_async_copy(o_hbm, o_hbm, sem_o.at[0]).wait()


@jax.jit
def pallas_standalone__conformer_conv_module__speech_kernel(
    x: jax.Array,
    w_pw1: jax.Array,
    dw: jax.Array,
    w_pw2: jax.Array,
):
    B, T, D = x.shape
    K = dw.shape[0]
    assert B == 2 and sum(CM2) == T and D % LANES == 0 and K // 2 <= GAP
    NL = D // LANES
    kern = functools.partial(_kernel, B=B, T=T, D=D, K=K)
    return pl.pallas_call(
        kern,
        in_specs=[pl.BlockSpec(memory_space=pl.ANY)] * 4,
        out_specs=pl.BlockSpec(memory_space=pl.ANY),
        out_shape=jax.ShapeDtypeStruct((B, T, D), x.dtype),
        scratch_shapes=[
            pltpu.VMEM((B, T, D), x.dtype),
            pltpu.VMEM((B, NL, T, LANES), x.dtype),
            pltpu.VMEM((2 * NL, D, LANES), w_pw1.dtype),
            pltpu.VMEM((NL, D, LANES), w_pw2.dtype),
            pltpu.VMEM((2 * NL, D // 2, LANES), jnp.uint32),
            pltpu.VMEM((NL, D // 2, LANES), jnp.uint32),
            pltpu.VMEM((K, D), dw.dtype),
            pltpu.VMEM((K, 8, D), jnp.float32),
            pltpu.VMEM((B, 2 * NL, HP, LANES), jnp.float32),
            pltpu.VMEM((NL, T + 3 * GAP, LANES), jnp.float32),
            pltpu.SemaphoreType.DMA((4 + B,)),
            pltpu.SemaphoreType.DMA((1,)),
        ],
        compiler_params=pltpu.CompilerParams(
            vmem_limit_bytes=100 * 1024 * 1024,
            disable_bounds_checks=True,
            disable_semaphore_checks=True),
    )(x, w_pw1, dw, w_pw2)
```
